```python
import os as _os
_os.environ.setdefault("JAX_PLATFORMS", "cpu")
import jax
import jax.numpy as jnp

def _softmax(x, axis=-1):
    return jax.nn.softmax(x, axis=axis)
def _gelu(x):
    return jax.nn.gelu(x, approximate=True)
def _silu(x):
    return jax.nn.silu(x)
def _sigmoid(x):
    return jax.nn.sigmoid(x)
def _layernorm(x, axis=-1, eps=1e-5):
    m = jnp.mean(x, axis=axis, keepdims=True)
    v = jnp.var(x, axis=axis, keepdims=True)
    return (x - m) / jnp.sqrt(v + eps)
def _scatter_add(tgt, idx, src, axis=0):
    return tgt.at[idx].add(src)
def _segment_sum(src, seg, n):
    return jax.ops.segment_sum(src, seg, n)
class _Rng:
    def __init__(self, key):
        self._k = key
    def _next(self):
        self._k, sub = jax.random.split(self._k)
        return sub
    def normal(self, shape):
        return jax.random.normal(self._next(), shape, dtype=jnp.bfloat16)
    def randint(self, lo, hi, shape):
        return jax.random.randint(self._next(), shape, lo, hi, dtype=jnp.int32)
    def uniform(self, shape, lo=0.0, hi=1.0):
        return jax.random.uniform(self._next(), shape, jnp.bfloat16, lo, hi)
    def permutation(self, n):
        return jax.random.permutation(self._next(), n)


kernel_name = 'parallel_sum__softmax_full_mha__swiglu_ffn__prompt'

def setup_inputs():
    _rng = _Rng(jax.random.key(int.from_bytes(__import__("os").urandom(4), "little")))
    _w = (lambda a: (lambda t: t.astype(jnp.bfloat16) if jnp.issubdtype(t.dtype, jnp.floating) else t)(jnp.asarray(a)))
    def _A_setup():
        B, S, D = 1, 2048, 640
        return {
            "x": _w((lambda *s: _rng.normal(s) * 0.05)(B, S, D)),
            "wqkv": _w((lambda *s: _rng.normal(s) * 0.1)(D, 3 * D)),
            "wo": _w((lambda *s: _rng.normal(s) * 0.05)(D, D)),
        }
    _A_in = _A_setup()

    def _B_setup():
        B, S, D, F = 1, 2048, 640, 1536
        return {
            "x": _w((lambda *s: _rng.normal(s) * 0.05)(B, S, D)),
            "w_gate": _w((lambda *s: _rng.normal(s) * 0.05)(D, F)),
            "w_up": _w((lambda *s: _rng.normal(s) * 0.05)(D, F)),
            "w_down": _w((lambda *s: _rng.normal(s) * 0.05)(F, D)),
        }
    _B_in = _B_setup()

    return {
        "A_x": _A_in["x"],
        "A_wqkv": _A_in["wqkv"],
        "A_wo": _A_in["wo"],
        "B_x": _B_in["x"],
        "B_w_gate": _B_in["w_gate"],
        "B_w_up": _B_in["w_up"],
        "B_w_down": _B_in["w_down"],
    }

def reference(A_x, A_wqkv, A_wo, B_x, B_w_gate, B_w_up, B_w_down):
    def _A_ref(x, wqkv, wo):
        B, S, D = x.shape
        H = 32; Dh = D // H
        qkv = (lambda x, *d: x.transpose(*d))((x @ wqkv).reshape(B, S, 3, H, Dh), 2, 0, 3, 1, 4)
        q, k, v = qkv[0], qkv[1], qkv[2]
        scale = Dh ** -0.5
        scores = jnp.einsum("bhqd,bhkd->bhqk", q, k) * scale
        p = _softmax(scores, axis=-1)
        o = jnp.einsum("bhqk,bhkd->bhqd", p, v)
        return (lambda x, *d: x.transpose(*d))(o, 0, 2, 1, 3).reshape(B, S, D) @ wo

    def _B_ref(x, w_gate, w_up, w_down):
        g = _silu(x @ w_gate)
        u = x @ w_up
        return (g * u) @ w_down

    x = A_x
    xn = _layernorm(x, axis=-1)
    return x + _A_ref(xn, A_wqkv, A_wo) + _B_ref(xn, B_w_gate, B_w_up, B_w_down)
```

```python
import functools
import math

import jax
import jax.numpy as jnp
from jax import lax
import jax.experimental.pallas as pl
import jax.experimental.pallas.tpu as pltpu

S = 2048
D = 640
H = 32
DH = 20
F = 1536
HPT = 6
NKT = 6
EPS = 1e-5
QSCALE = (DH ** -0.5) * math.log2(math.e)

_NT = (((1,), (1,)), ((), ()))
_TN = (((0,), (0,)), ((), ()))


def _kernel(x_hbm, wqkv_hbm, wo_hbm, wg_hbm, wu_hbm, wd_hbm, out_hbm,
            x_ref, wqkv_ref, wo_ref, wg_ref, wu_ref, wd_ref, out_ref,
            xn_ref, wk_ref, wqvt_ref, k_ref, qt_ref, vt_ref, ot_ref,
            s0_ref, s1_ref, m0_ref, m1_ref, sem_x, sem_w, sem_o,
            *, tq, ck, hpb, order, lag):
    f32 = jnp.float32
    bf16 = jnp.bfloat16
    tr = tq
    nqt = S // tq
    nck = S // ck

    def x_copy(t):
        return pltpu.make_async_copy(x_hbm.at[pl.ds(t * tr, tr), :], x_ref.at[pl.ds(t * tr, tr), :], sem_x.at[t])

    def o_copy(t):
        return pltpu.make_async_copy(out_ref.at[pl.ds(t * tr, tr), :], out_hbm.at[pl.ds(t * tr, tr), :], sem_o.at[t])

    w_copies = [pltpu.make_async_copy(src, dst, sem_w.at[n]) for n, (src, dst) in enumerate(
        [(wqkv_hbm, wqkv_ref), (wo_hbm, wo_ref), (wg_hbm, wg_ref), (wu_hbm, wu_ref), (wd_hbm, wd_ref)])]

    x_copy(0).start()
    w_copies[0].start()
    for t in range(1, nqt):
        x_copy(t).start()
    for cp in w_copies[1:]:
        cp.start()

    def layer_norm(t):
        x = x_ref[t * tr:(t + 1) * tr, :].astype(f32)
        mean = jnp.mean(x, axis=-1, keepdims=True)
        xc = x - mean
        var = jnp.mean(xc * xc, axis=-1, keepdims=True)
        xn_ref[t * tr:(t + 1) * tr, :] = (xc * lax.rsqrt(var + EPS)).astype(bf16)

    x_copy(0).wait()
    layer_norm(0)
    w_copies[0].wait()
    for j in range(NKT):
        wk_ref[:, j * 128:(j + 1) * 128] = wqkv_ref[:, D + 120 * j:D + 120 * j + 128]
    wqvt_ref[0:D, :] = wqkv_ref[:, 0:D].T
    wqvt_ref[D:2 * D, :] = wqkv_ref[:, 2 * D:3 * D].T

    row32 = lax.broadcasted_iota(jnp.int32, (32, tr), 0)

    for t in range(nqt):
        if t + 1 < nqt:
            x_copy(t + 1).wait()
            layer_norm(t + 1)
        xn = xn_ref[t * tr:(t + 1) * tr, :]
        kk = jnp.dot(xn, wk_ref[...], preferred_element_type=f32).astype(bf16)
        for j in range(NKT):
            k_ref[j, t * tr:(t + 1) * tr, :] = kk[:, j * 128:(j + 1) * 128]
        qv = lax.dot_general(wqvt_ref[...], xn, _NT, preferred_element_type=f32)
        qt_ref[t, 0:D, :] = qv[0:D] * QSCALE
        qt_ref[t, D:768, :] = jnp.zeros((768 - D, tr), f32)
        for h in range(H):
            w = 16 * ((DH * h) // 16)
            off = DH * h - w
            r = 0 if off == 12 else 31
            win = qv[D + w:D + w + 32]
            vt_ref[h, :, t * tr:(t + 1) * tr] = jnp.where(row32 == r, 1.0, win).astype(bf16)
        ot_ref[t] = jnp.zeros((D, tq), f32)

    row128 = lax.broadcasted_iota(jnp.int32, (128, tq), 0)
    row32q = lax.broadcasted_iota(jnp.int32, (32, tq), 0)

    def q_weights(h, t):
        j = h // HPT
        o = DH * (h % HPT)
        win = qt_ref[t, pl.ds(pl.multiple_of(120 * j, 8), 128), :]
        mask = (row128 >= o) & (row128 < o + DH)
        return jnp.where(mask, win, 0.0).astype(bf16), j

    def qk_chunk(wq, j, c, s_ref, mx):
        s = jnp.dot(k_ref[j, c * ck:(c + 1) * ck, :], wq, preferred_element_type=f32)
        s_ref[c * ck:(c + 1) * ck, :] = s
        return jnp.maximum(mx, jnp.max(s.reshape(ck // 8, 8, tq), axis=0))

    def pv_chunk(h, c, s_ref, m, acc):
        p = jnp.exp2(s_ref[c * ck:(c + 1) * ck, :] - m).astype(bf16)
        return acc + jnp.dot(vt_ref[h, :, c * ck:(c + 1) * ck], p, preferred_element_type=f32)

    def finish(h, t, acc):
        w = 16 * ((DH * h) // 16)
        off = DH * h - w
        if isinstance(h, int):
            den = acc[0:1] if off == 12 else acc[31:32]
        else:
            w = pl.multiple_of(w, 16)
            den = jnp.where(off == 12, acc[0:1], acc[31:32])
        o = acc * (1.0 / den)
        mask = (row32q >= off) & (row32q < off + DH)
        ot_ref[t, pl.ds(w, 32), :] = jnp.where(mask, o, ot_ref[t, pl.ds(w, 32), :])

    neg = jnp.full((8, tq), -jnp.inf, f32)
    bufs = ((s0_ref, m0_ref), (s1_ref, m1_ref))

    def stream(curs, nxts):
        n_items = max(len(curs), len(nxts))
        qk_state = None
        pv_state = None
        for g in range(n_items * nck + lag):
            n, c = divmod(g, nck)
            if n < len(nxts):
                s_nxt, m_nxt = bufs[(n + 1) % 2]
                if c == 0:
                    wq, j = q_weights(*nxts[n])
                    mx = neg
                mx = qk_chunk(wq, j, c, s_nxt, mx)
                if c == nck - 1:
                    m_nxt[...] = jnp.max(mx, axis=0, keepdims=True)
            n, c = divmod(g - lag, nck)
            if 0 <= n < len(curs):
                s_cur, m_cur = bufs[n % 2]
                if c == 0:
                    m = m_cur[...]
                    acc = jnp.zeros((32, tq), f32)
                acc = pv_chunk(curs[n][0], c, s_cur, m, acc)
                if c == nck - 1:
                    finish(curs[n][0], curs[n][1], acc)

    wq, j = q_weights(0, 0)
    mx = neg
    for c in range(nck):
        mx = qk_chunk(wq, j, c, s0_ref, mx)
    m0_ref[...] = jnp.max(mx, axis=0, keepdims=True)

    per_body = hpb * nqt

    def body_items(hb):
        items = [(hb * hpb + a, t) for a in range(hpb) for t in range(nqt)]
        return items + [(hb * hpb + hpb, 0)]

    def attn_body(hb, carry):
        items = body_items(hb)
        stream(items[:-1], items[1:])
        return carry

    nb = H // hpb
    lax.fori_loop(0, nb - 1, attn_body, 0)
    items = body_items(nb - 1)
    stream(items[:-1], items[1:-1])

    for cp in w_copies[1:]:
        cp.wait()

    def out_body(t, carry):
        r0 = pl.multiple_of(t * tr, tr)
        xn = xn_ref[pl.ds(r0, tr), :]
        attn = lax.dot_general(ot_ref[t].astype(bf16), wo_ref[...], _TN, preferred_element_type=f32)
        g = jnp.dot(xn, wg_ref[...], preferred_element_type=f32)
        u = jnp.dot(xn, wu_ref[...], preferred_element_type=f32)
        hm = (g * jax.nn.sigmoid(g) * u).astype(bf16)
        ffn = jnp.dot(hm, wd_ref[...], preferred_element_type=f32)
        x = x_ref[pl.ds(r0, tr), :].astype(f32)
        out_ref[pl.ds(r0, tr), :] = (x + attn + ffn).astype(bf16)
        o_copy(t).start()
        return carry

    lax.fori_loop(0, nqt, out_body, 0)
    for t in range(nqt):
        o_copy(t).wait()


@jax.jit
def pallas_parallel_sum__softmax_full_mha__swiglu_ffn__prompt_kernel(
        A_x, A_wqkv, A_wo, B_x, B_w_gate, B_w_up, B_w_down):
    tq, ck, hpb, order, lag = 512, 128, 2, 0, 2
    del B_x
    bf16 = jnp.bfloat16
    f32 = jnp.float32
    nqt = S // tq
    x = A_x.reshape(S, D)
    any_spec = pl.BlockSpec(memory_space=pl.ANY)
    out = pl.pallas_call(
        functools.partial(_kernel, tq=tq, ck=ck, hpb=hpb, order=order, lag=lag),
        out_shape=jax.ShapeDtypeStruct((S, D), bf16),
        in_specs=[any_spec] * 6,
        out_specs=any_spec,
        scratch_shapes=[
            pltpu.VMEM((S, D), bf16),
            pltpu.VMEM((D, 3 * D), bf16),
            pltpu.VMEM((D, D), bf16),
            pltpu.VMEM((D, F), bf16),
            pltpu.VMEM((D, F), bf16),
            pltpu.VMEM((F, D), bf16),
            pltpu.VMEM((S, D), bf16),
            pltpu.VMEM((S, D), bf16),
            pltpu.VMEM((D, NKT * 128), bf16),
            pltpu.VMEM((2 * D, D), bf16),
            pltpu.VMEM((NKT, S, 128), bf16),
            pltpu.VMEM((nqt, 768, tq), f32),
            pltpu.VMEM((H, 32, S), bf16),
            pltpu.VMEM((nqt, D, tq), f32),
            pltpu.VMEM((S, tq), f32),
            pltpu.VMEM((S, tq), f32),
            pltpu.VMEM((1, tq), f32),
            pltpu.VMEM((1, tq), f32),
            pltpu.SemaphoreType.DMA((nqt,)),
            pltpu.SemaphoreType.DMA((5,)),
            pltpu.SemaphoreType.DMA((nqt,)),
        ],
        compiler_params=pltpu.CompilerParams(vmem_limit_bytes=110 * 1024 * 1024),
    )(x, A_wqkv, A_wo, B_w_gate, B_w_up, B_w_down)
    return out.reshape(1, S, D)
```

```python
import functools
import math

import jax
import jax.numpy as jnp
from jax import lax
import jax.experimental.pallas as pl
import jax.experimental.pallas.tpu as pltpu

S = 2048
D = 640
H = 32
DH = 20
F = 1536
EPS = 1e-5
QSCALE = (DH ** -0.5) * math.log2(math.e)

HPT = 6
NKT = 6
KX = 48
VW = 24
TQ = 512
CK = 128
HPB = 2
LAG = 2
RA = 384
OSPLIT = 4

NQT = S // TQ
NCK = S // CK

_NT = (((1,), (1,)), ((), ()))
_TN = (((0,), (0,)), ((), ()))


def _kernel(x_hbm, wqkv_hbm, wo_hbm, wg_hbm, wu_hbm, wd_hbm, out_hbm,
            x_ref, wqkv_ref, wo_ref, wg_ref, wu_ref, wd_ref, out_ref,
            xn_ref, wk_ref, wqvt_ref, k_ref, qt_ref, vt_ref, ot_ref, part_ref,
            s0_ref, s1_ref, m0_ref, m1_ref, z_ref, sem_x, sem_w, sem_o):
    f32 = jnp.float32
    bf16 = jnp.bfloat16

    def x_rows(n, lo, hi):
        return pltpu.make_async_copy(x_hbm.at[lo:hi, :], x_ref.at[lo:hi, :], sem_x.at[n])

    def w_cols(n, lo, hi):
        return pltpu.make_async_copy(wqkv_hbm.at[:, lo:hi], wqkv_ref.at[:, lo:hi], sem_w.at[n])

    def o_rows(n, lo, hi):
        return pltpu.make_async_copy(out_ref.at[lo:hi, :], out_hbm.at[lo:hi, :], sem_o.at[n])

    xa_copy = x_rows(0, 0, RA)
    xb_copy = x_rows(1, RA, TQ)
    x_copies = [x_rows(1 + t, t * TQ, (t + 1) * TQ) for t in range(1, NQT)]
    wka_copy = w_cols(0, D, D + 384)
    wkb_copy = w_cols(1, D + 384, 2 * D)
    wq_copy = w_cols(2, 0, D)
    wv_copy = w_cols(3, 2 * D, 3 * D)
    late_copies = [
        pltpu.make_async_copy(src, dst, sem_w.at[4 + n])
        for n, (src, dst) in enumerate(
            [(wg_hbm, wg_ref), (wu_hbm, wu_ref), (wd_hbm, wd_ref), (wo_hbm, wo_ref)])
    ]

    z_ref[0] = 0
    for cp in [xa_copy, wka_copy, xb_copy, wkb_copy] + x_copies + [wq_copy, wv_copy]:
        cp.start()

    def layer_norm(lo, hi):
        x = x_ref[lo:hi, :].astype(f32)
        mean = jnp.mean(x, axis=-1, keepdims=True)
        xc = x - mean
        var = jnp.mean(xc * xc, axis=-1, keepdims=True)
        xn_ref[lo:hi, :] = (xc * lax.rsqrt(var + EPS)).astype(bf16)

    def wk_prep(j0, j1):
        for j in range(j0, j1):
            wk_ref[:, j * 128:(j + 1) * 128] = wqkv_ref[:, D + 120 * j:D + 120 * j + 128]

    def k_proj(lo, hi, j0, j1):
        kk = jnp.dot(xn_ref[lo:hi, :], wk_ref[:, j0 * 128:j1 * 128],
                     preferred_element_type=f32).astype(bf16)
        for j in range(j0, j1):
            k_ref[j, lo:hi, :] = kk[:, (j - j0) * 128:(j - j0 + 1) * 128]

    def k_proj_all(lo, hi):
        k_proj(lo, hi, 0, 4)
        q = (hi - lo) // 4
        for p in range(4):
            k_proj(lo + p * q, lo + (p + 1) * q, 4, 5)

    row24 = lax.broadcasted_iota(jnp.int32, (VW, TQ), 0)

    def qv_proj(t):
        lo, hi = t * TQ, (t + 1) * TQ
        qv = lax.dot_general(wqvt_ref[0:2 * D + KX, :], xn_ref[lo:hi, :], _NT,
                             preferred_element_type=f32)
        qt_ref[t, 0:D, :] = qv[0:D] * QSCALE
        for h in range(H):
            w = 8 * ((DH * h) // 8)
            ones_row = 0 if h % 2 else VW - 1
            vt_ref[h, :, lo:hi] = jnp.where(row24 == ones_row, 1.0, qv[D + w:D + w + VW])
        kx = jnp.concatenate([qv[2 * D:2 * D + KX], jnp.zeros((128 - KX, TQ), f32)], axis=0)
        k_ref[NKT - 1, lo:hi, :] = kx.T.astype(bf16)

    xa_copy.wait()
    layer_norm(0, RA)
    wka_copy.wait()
    wk_prep(0, 3)
    k_proj(0, RA, 0, 3)
    xb_copy.wait()
    wkb_copy.wait()
    layer_norm(RA, TQ)
    wk_prep(3, 5)
    k_proj(0, RA, 3, 5)
    x_copies[0].wait()
    k_proj_all(RA, TQ)
    layer_norm(TQ, 2 * TQ)
    for t in range(1, NQT - 1):
        x_copies[t].wait()
        k_proj_all(t * TQ, (t + 1) * TQ)
        layer_norm((t + 1) * TQ, (t + 2) * TQ)
    wq_copy.wait()
    wv_copy.wait()
    for cp in late_copies:
        cp.start()
    k_proj_all((NQT - 1) * TQ, NQT * TQ)
    wqvt_ref[0:D, :] = wqkv_ref[:, 0:D].T
    wqvt_ref[D:2 * D, :] = wqkv_ref[:, 2 * D:3 * D].T
    wqvt_ref[2 * D:2 * D + KX, :] = wqkv_ref[:, 2 * D - 128:2 * D].T[128 - KX:128]
    for t in range(NQT):
        qv_proj(t)
    for cp in late_copies:
        cp.wait()

    def ffn_body(t, carry):
        r0 = pl.multiple_of(t * TQ, TQ)
        xn = xn_ref[pl.ds(r0, TQ), :]
        g = jnp.dot(xn, wg_ref[...], preferred_element_type=f32)
        u = jnp.dot(xn, wu_ref[...], preferred_element_type=f32)
        hm = (g * jax.nn.sigmoid(g) * u).astype(bf16)
        ffn = jnp.dot(hm, wd_ref[...], preferred_element_type=f32)
        part_ref[pl.ds(r0, TQ), :] = x_ref[pl.ds(r0, TQ), :].astype(f32) + ffn
        s1_ref[pl.ds(r0, TQ), :] = jnp.zeros((TQ, TQ), f32)
        m1_ref[...] = jnp.zeros((1, TQ), f32)
        return carry

    lax.fori_loop(0, NQT, ffn_body, 0)

    row128 = lax.broadcasted_iota(jnp.int32, (128, TQ), 0)
    row8 = lax.broadcasted_iota(jnp.int32, (8, TQ), 0)

    def q_weights(h, t):
        j = h // HPT
        start = jnp.minimum(120 * j, D - KX)
        o = DH * h - start
        win = qt_ref[t, pl.ds(pl.multiple_of(start, 8), 128), :]
        mask = (row128 >= o) & (row128 < o + DH)
        return jnp.where(mask, win, 0.0).astype(bf16), j

    def qk_chunk(wq, j, c, s_ref, mx):
        s = jnp.dot(k_ref[j, c * CK:(c + 1) * CK, :], wq, preferred_element_type=f32)
        s_ref[c * CK:(c + 1) * CK, :] = s
        return jnp.maximum(mx, jnp.max(s.reshape(CK // 8, 8, TQ), axis=0))

    def pv_chunk(h, c, s_ref, m, acc):
        p = jnp.exp2(s_ref[c * CK:(c + 1) * CK, :] - m).astype(bf16)
        return acc + jnp.dot(vt_ref[h, :, c * CK:(c + 1) * CK], p, preferred_element_type=f32)

    def finish(h, t, odd, acc):
        w = DH * h - (4 if odd else 0)
        if not isinstance(h, int):
            w = pl.multiple_of(w, 8)
        den = acc[0:1] if odd else acc[VW - 1:VW]
        o = acc * (1.0 / den)
        if odd:
            pltpu.store(ot_ref.at[t, pl.ds(w, 8), :], o[0:8], mask=row8 >= 4)
            ot_ref[t, pl.ds(w + 8, 16), :] = o[8:VW]
        else:
            ot_ref[t, pl.ds(w, 16), :] = o[0:16]
            pltpu.store(ot_ref.at[t, pl.ds(w + 16, 8), :], o[16:VW], mask=row8 < 4)

    neg = jnp.full((8, TQ), -jnp.inf, f32)
    bufs = ((s0_ref, m0_ref), (s1_ref, m1_ref))

    def stream(curs, nxts):
        n_items = max(len(curs), len(nxts))
        for g in range(n_items * NCK + LAG):
            n, c = divmod(g, NCK)
            if n < len(nxts):
                s_nxt, m_nxt = bufs[n % 2]
                if c == 0:
                    wq, j = q_weights(nxts[n][0], nxts[n][1])
                    mx = neg
                mx = qk_chunk(wq, j, c, s_nxt, mx)
                if c == NCK - 1:
                    m_nxt[...] = jnp.max(mx, axis=0, keepdims=True)
            n, c = divmod(g - LAG, NCK)
            if 0 <= n < len(curs):
                s_cur, m_cur = bufs[(n + 1) % 2]
                if c == 0:
                    m = m_cur[...]
                    acc = jnp.zeros((VW, TQ), f32)
                acc = pv_chunk(curs[n][0], c, s_cur, m, acc)
                if c == NCK - 1:
                    finish(*curs[n], acc)

    def attn_body(hb, carry):
        items = [(hb * HPB + a, t, a % 2 == 1) for a in range(HPB) for t in range(NQT)]
        prev = (jnp.maximum(hb * HPB - 1, 1), NQT - 1, True)
        stream([prev] + items[:-1], items)
        return carry

    lax.fori_loop(0, H // HPB, attn_body, 0)

    z = z_ref[0]
    m1_ref[...] = jnp.where(z == 0, m1_ref[...], s0_ref[pl.ds(pl.multiple_of(8 * z, 8), 1), :])
    stream([(H - 1, NQT - 1, True)], [])

    copies = []
    for t in range(NQT):
        parts = OSPLIT if t == NQT - 1 else 1
        rows = TQ // parts
        for p in range(parts):
            lo = t * TQ + p * rows
            o_t = ot_ref[t, :, p * rows:(p + 1) * rows].astype(bf16)
            attn = lax.dot_general(o_t, wo_ref[...], _TN, preferred_element_type=f32)
            out_ref[lo:lo + rows, :] = (part_ref[lo:lo + rows, :] + attn).astype(bf16)
            cp = o_rows(len(copies), lo, lo + rows)
            cp.start()
            copies.append(cp)
    for cp in copies:
        cp.wait()


@jax.jit
def pallas_parallel_sum__softmax_full_mha__swiglu_ffn__prompt_kernel(
    A_x: jax.Array,
    A_wqkv: jax.Array,
    A_wo: jax.Array,
    B_x: jax.Array,
    B_w_gate: jax.Array,
    B_w_up: jax.Array,
    B_w_down: jax.Array,
):
    del B_x
    bf16 = jnp.bfloat16
    f32 = jnp.float32
    any_spec = pl.BlockSpec(memory_space=pl.ANY)
    out = pl.pallas_call(
        _kernel,
        out_shape=jax.ShapeDtypeStruct((S, D), bf16),
        in_specs=[any_spec] * 6,
        out_specs=any_spec,
        scratch_shapes=[
            pltpu.VMEM((S, D), bf16),
            pltpu.VMEM((D, 3 * D), bf16),
            pltpu.VMEM((D, D), bf16),
            pltpu.VMEM((D, F), bf16),
            pltpu.VMEM((D, F), bf16),
            pltpu.VMEM((F, D), bf16),
            pltpu.VMEM((S, D), bf16),
            pltpu.VMEM((S, D), bf16),
            pltpu.VMEM((D, (NKT - 1) * 128), bf16),
            pltpu.VMEM((2 * D + 64, D), bf16),
            pltpu.VMEM((NKT, S, 128), bf16),
            pltpu.VMEM((NQT, 768, TQ), f32),
            pltpu.VMEM((H, VW, S), f32),
            pltpu.VMEM((NQT, D, TQ), f32),
            pltpu.VMEM((S, D), f32),
            pltpu.VMEM((S, TQ), f32),
            pltpu.VMEM((S, TQ), f32),
            pltpu.VMEM((1, TQ), f32),
            pltpu.VMEM((1, TQ), f32),
            pltpu.SMEM((1,), jnp.int32),
            pltpu.SemaphoreType.DMA((NQT + 1,)),
            pltpu.SemaphoreType.DMA((8,)),
            pltpu.SemaphoreType.DMA((NQT - 1 + OSPLIT,)),
        ],
        compiler_params=pltpu.CompilerParams(vmem_limit_bytes=110 * 1024 * 1024),
    )(A_x.reshape(S, D), A_wqkv, A_wo, B_w_gate, B_w_up, B_w_down)
    return out.reshape(1, S, D)
```

```python
import math

import jax
import jax.numpy as jnp
from jax import lax
import jax.experimental.pallas as pl
import jax.experimental.pallas.tpu as pltpu

S = 2048
D = 640
H = 32
DH = 20
F = 1536
EPS = 1e-5
QSCALE = (DH ** -0.5) * math.log2(math.e)

HPT = 6
NKT = 6
KX = 48
VW = 24
TQ = 512
CK = 128
HPB = 2
LAG = 2
RA = 384
OSPLIT = 4

NQT = S // TQ
NCK = S // CK
FR = S // (H // HPB)

_NT = (((1,), (1,)), ((), ()))
_TN = (((0,), (0,)), ((), ()))


def _kernel(x_hbm, wqkv_hbm, wo_hbm, wg_hbm, wu_hbm, wd_hbm, out_hbm,
            x_ref, wqkv_ref, wo_ref, wg_ref, wu_ref, wd_ref, out_ref,
            xn_ref, wk_ref, wqvt_ref, k_ref, qt_ref, vt_ref, ot_ref, part_ref,
            s0_ref, s1_ref, m0_ref, m1_ref, z_ref, sem_x, sem_w, sem_o):
    f32 = jnp.float32
    bf16 = jnp.bfloat16

    def x_rows(n, lo, hi):
        return pltpu.make_async_copy(x_hbm.at[lo:hi, :], x_ref.at[lo:hi, :], sem_x.at[n])

    def w_cols(n, lo, hi):
        return pltpu.make_async_copy(wqkv_hbm.at[:, lo:hi], wqkv_ref.at[:, lo:hi], sem_w.at[n])

    def o_rows(n, lo, hi):
        return pltpu.make_async_copy(out_ref.at[lo:hi, :], out_hbm.at[lo:hi, :], sem_o.at[n])

    xa_copy = x_rows(0, 0, RA)
    xb_copy = x_rows(1, RA, TQ)
    x_copies = [x_rows(1 + t, t * TQ, (t + 1) * TQ) for t in range(1, NQT)]
    wka_copy = w_cols(0, D, D + 384)
    wkb_copy = w_cols(1, D + 384, 2 * D)
    wq_copy = w_cols(2, 0, D)
    wv_copy = w_cols(3, 2 * D, 3 * D)
    late_copies = [
        pltpu.make_async_copy(src, dst, sem_w.at[4 + n])
        for n, (src, dst) in enumerate(
            [(wg_hbm, wg_ref), (wu_hbm, wu_ref), (wd_hbm, wd_ref), (wo_hbm, wo_ref)])
    ]

    z_ref[0] = 0
    for cp in [xa_copy, wka_copy, xb_copy, wkb_copy] + x_copies + [wq_copy, wv_copy]:
        cp.start()

    def layer_norm(lo, hi):
        x = x_ref[lo:hi, :].astype(f32)
        mean = jnp.mean(x, axis=-1, keepdims=True)
        xc = x - mean
        var = jnp.mean(xc * xc, axis=-1, keepdims=True)
        xn_ref[lo:hi, :] = (xc * lax.rsqrt(var + EPS)).astype(bf16)

    def wk_prep(j0, j1):
        for j in range(j0, j1):
            wk_ref[:, j * 128:(j + 1) * 128] = wqkv_ref[:, D + 120 * j:D + 120 * j + 128]

    def k_proj(lo, hi, j0, j1):
        kk = jnp.dot(xn_ref[lo:hi, :], wk_ref[:, j0 * 128:j1 * 128],
                     preferred_element_type=f32).astype(bf16)
        for j in range(j0, j1):
            k_ref[j, lo:hi, :] = kk[:, (j - j0) * 128:(j - j0 + 1) * 128]

    def k_split(lo, hi, j0, j1, parts):
        q = (hi - lo) // parts
        for p in range(parts):
            k_proj(lo + p * q, lo + (p + 1) * q, j0, j1)

    row24 = lax.broadcasted_iota(jnp.int32, (VW, TQ), 0)

    def qv_proj(t):
        lo, hi = t * TQ, (t + 1) * TQ
        qv = lax.dot_general(wqvt_ref[0:2 * D + KX, :], xn_ref[lo:hi, :], _NT,
                             preferred_element_type=f32)
        qt_ref[t, 0:D, :] = qv[0:D] * QSCALE
        for h in range(H):
            w = 8 * ((DH * h) // 8)
            ones_row = 0 if h % 2 else VW - 1
            vt_ref[h, :, lo:hi] = jnp.where(row24 == ones_row, 1.0, qv[D + w:D + w + VW])
        kx = jnp.concatenate([jnp.zeros((128 - KX, TQ), f32), qv[2 * D:2 * D + KX]], axis=0)
        k_ref[NKT - 1, lo:hi, :] = kx.T.astype(bf16)

    s1_ref[...] = jnp.zeros((S, TQ), f32)
    m1_ref[...] = jnp.zeros((1, TQ), f32)

    xa_copy.wait()
    layer_norm(0, RA)
    wka_copy.wait()
    wk_prep(0, 3)
    k_proj(0, RA, 0, 3)
    xb_copy.wait()
    wkb_copy.wait()
    layer_norm(RA, TQ)
    wk_prep(3, 5)
    k_proj(0, RA, 3, 5)
    for t in range(1, NQT):
        x_copies[t - 1].wait()
        if t == 1:
            k_proj(RA, TQ, 0, 4)
            k_split(RA, TQ, 4, 5, 4)
        else:
            k_split((t - 1) * TQ, t * TQ, 3, 5, 2)
        layer_norm(t * TQ, (t + 1) * TQ)
        k_split(t * TQ, (t + 1) * TQ, 0, 3, 4)
    wq_copy.wait()
    wv_copy.wait()
    for cp in late_copies:
        cp.start()
    k_split((NQT - 1) * TQ, NQT * TQ, 3, 5, 2)
    wqvt_ref[0:D, :] = wqkv_ref[:, 0:D].T
    wqvt_ref[D:2 * D, :] = wqkv_ref[:, 2 * D:3 * D].T
    wqvt_ref[2 * D:2 * D + KX, :] = wqkv_ref[:, 2 * D - 128:2 * D].T[128 - KX:128]
    for t in range(NQT):
        qv_proj(t)
    for cp in late_copies:
        cp.wait()

    row128 = lax.broadcasted_iota(jnp.int32, (128, TQ), 0)
    row8 = lax.broadcasted_iota(jnp.int32, (8, TQ), 0)

    def q_weights(h, t):
        j = h // HPT
        start = jnp.minimum(120 * j, D - 128)
        o = DH * h - start
        win = qt_ref[t, pl.ds(pl.multiple_of(start, 8), 128), :]
        mask = (row128 >= o) & (row128 < o + DH)
        return jnp.where(mask, win, 0.0).astype(bf16), j

    def qk_chunk(wq, j, c, s_ref, mx):
        s = jnp.dot(k_ref[j, c * CK:(c + 1) * CK, :], wq, preferred_element_type=f32)
        s_ref[c * CK:(c + 1) * CK, :] = s
        return jnp.maximum(mx, jnp.max(s.reshape(CK // 8, 8, TQ), axis=0))

    def pv_chunk(h, c, s_ref, m, acc):
        p = jnp.exp2(s_ref[c * CK:(c + 1) * CK, :] - m).astype(bf16)
        return acc + jnp.dot(vt_ref[h, :, c * CK:(c + 1) * CK], p, preferred_element_type=f32)

    def finish(h, t, odd, acc):
        w = DH * h - (4 if odd else 0)
        if not isinstance(h, int):
            w = pl.multiple_of(w, 8)
        den = acc[0:1] if odd else acc[VW - 1:VW]
        o = acc * (1.0 / den)
        if odd:
            pltpu.store(ot_ref.at[t, pl.ds(w, 8), :], o[0:8], mask=row8 >= 4)
            ot_ref[t, pl.ds(w + 8, 16), :] = o[8:VW]
        else:
            ot_ref[t, pl.ds(w, 16), :] = o[0:16]
            pltpu.store(ot_ref.at[t, pl.ds(w + 16, 8), :], o[16:VW], mask=row8 < 4)

    neg = jnp.full((8, TQ), -jnp.inf, f32)
    bufs = ((s0_ref, m0_ref), (s1_ref, m1_ref))

    def stream(curs, nxts):
        n_items = max(len(curs), len(nxts))
        for g in range(n_items * NCK + LAG):
            n, c = divmod(g, NCK)
            if n < len(nxts):
                s_nxt, m_nxt = bufs[n % 2]
                if c == 0:
                    wq, j = q_weights(nxts[n][0], nxts[n][1])
                    mx = neg
                mx = qk_chunk(wq, j, c, s_nxt, mx)
                if c == NCK - 1:
                    m_nxt[...] = jnp.max(mx, axis=0, keepdims=True)
            n, c = divmod(g - LAG, NCK)
            if 0 <= n < len(curs):
                s_cur, m_cur = bufs[(n + 1) % 2]
                if c == 0:
                    m = m_cur[...]
                    acc = jnp.zeros((VW, TQ), f32)
                acc = pv_chunk(curs[n][0], c, s_cur, m, acc)
                if c == NCK - 1:
                    finish(*curs[n], acc)

    def attn_body(hb, carry):
        r0 = pl.multiple_of(hb * FR, FR)
        xn = xn_ref[pl.ds(r0, FR), :]
        g = jnp.dot(xn, wg_ref[...], preferred_element_type=f32)
        u = jnp.dot(xn, wu_ref[...], preferred_element_type=f32)
        hm = (g * jax.nn.sigmoid(g) * u).astype(bf16)

        items = [(hb * HPB + a, t, a % 2 == 1) for a in range(HPB) for t in range(NQT)]
        prev = (jnp.maximum(hb * HPB - 1, 1), NQT - 1, True)
        stream([prev] + items[:-1], items)

        ffn = jnp.dot(hm, wd_ref[...], preferred_element_type=f32)
        part_ref[pl.ds(r0, FR), :] = x_ref[pl.ds(r0, FR), :].astype(f32) + ffn
        return carry

    lax.fori_loop(0, H // HPB, attn_body, 0)

    z = z_ref[0]
    m1_ref[...] = jnp.where(z == 0, m1_ref[...], s0_ref[pl.ds(pl.multiple_of(8 * z, 8), 1), :])
    stream([(H - 1, NQT - 1, True)], [])

    copies = []
    for t in range(NQT):
        parts = OSPLIT if t == NQT - 1 else 1
        rows = TQ // parts
        for p in range(parts):
            lo = t * TQ + p * rows
            o_t = ot_ref[t, :, p * rows:(p + 1) * rows].astype(bf16)
            attn = lax.dot_general(o_t, wo_ref[...], _TN, preferred_element_type=f32)
            out_ref[lo:lo + rows, :] = (part_ref[lo:lo + rows, :] + attn).astype(bf16)
            cp = o_rows(len(copies), lo, lo + rows)
            cp.start()
            copies.append(cp)
    for cp in copies:
        cp.wait()


@jax.jit
def pallas_parallel_sum__softmax_full_mha__swiglu_ffn__prompt_kernel(
    A_x: jax.Array,
    A_wqkv: jax.Array,
    A_wo: jax.Array,
    B_x: jax.Array,
    B_w_gate: jax.Array,
    B_w_up: jax.Array,
    B_w_down: jax.Array,
):
    del B_x
    bf16 = jnp.bfloat16
    f32 = jnp.float32
    any_spec = pl.BlockSpec(memory_space=pl.ANY)
    out = pl.pallas_call(
        _kernel,
        out_shape=jax.ShapeDtypeStruct((S, D), bf16),
        in_specs=[any_spec] * 6,
        out_specs=any_spec,
        scratch_shapes=[
            pltpu.VMEM((S, D), bf16),
            pltpu.VMEM((D, 3 * D), bf16),
            pltpu.VMEM((D, D), bf16),
            pltpu.VMEM((D, F), bf16),
            pltpu.VMEM((D, F), bf16),
            pltpu.VMEM((F, D), bf16),
            pltpu.VMEM((S, D), bf16),
            pltpu.VMEM((S, D), bf16),
            pltpu.VMEM((D, (NKT - 1) * 128), bf16),
            pltpu.VMEM((2 * D + 64, D), bf16),
            pltpu.VMEM((NKT, S, 128), bf16),
            pltpu.VMEM((NQT, D, TQ), f32),
            pltpu.VMEM((H, VW, S), f32),
            pltpu.VMEM((NQT, D, TQ), f32),
            pltpu.VMEM((S, D), f32),
            pltpu.VMEM((S, TQ), f32),
            pltpu.VMEM((S, TQ), f32),
            pltpu.VMEM((1, TQ), f32),
            pltpu.VMEM((1, TQ), f32),
            pltpu.SMEM((1,), jnp.int32),
            pltpu.SemaphoreType.DMA((NQT + 1,)),
            pltpu.SemaphoreType.DMA((8,)),
            pltpu.SemaphoreType.DMA((NQT - 1 + OSPLIT,)),
        ],
        compiler_params=pltpu.CompilerParams(vmem_limit_bytes=110 * 1024 * 1024),
    )(A_x.reshape(S, D), A_wqkv, A_wo, B_w_gate, B_w_up, B_w_down)
    return out.reshape(1, S, D)
```

```python
import math

import jax
import jax.numpy as jnp
from jax import lax
import jax.experimental.pallas as pl
import jax.experimental.pallas.tpu as pltpu

S = 2048
D = 640
H = 32
DH = 20
F = 1536
EPS = 1e-5
QSCALE = (DH ** -0.5) * math.log2(math.e)

HPT = 6
NKT = 6
KX = 48
VW = 24
TQ = 512
CK = 128
HPB = 2
LAG = 2
RA = 384
OSPLIT = 4

NQT = S // TQ
NCK = S // CK
FR = S // (H // HPB)
FQ = F // 4

_NT = (((1,), (1,)), ((), ()))
_TN = (((0,), (0,)), ((), ()))


def _kernel(x_hbm, wqkv_hbm, wo_hbm, wg_hbm, wu_hbm, wd_hbm, out_hbm,
            x_ref, wqkv_ref, wo_ref, wg_ref, wu_ref, wd_ref, out_ref,
            xn_ref, wk_ref, wqvt_ref, k_ref, qt_ref, vt_ref, ot_ref, part_ref,
            s0_ref, s1_ref, m0_ref, m1_ref, z_ref, sem_x, sem_w, sem_o):
    f32 = jnp.float32
    bf16 = jnp.bfloat16

    def x_rows(n, lo, hi):
        return pltpu.make_async_copy(x_hbm.at[lo:hi, :], x_ref.at[lo:hi, :], sem_x.at[n])

    def w_cols(n, lo, hi):
        return pltpu.make_async_copy(wqkv_hbm.at[:, lo:hi], wqkv_ref.at[:, lo:hi], sem_w.at[n])

    def o_rows(n, lo, hi):
        return pltpu.make_async_copy(out_ref.at[lo:hi, :], out_hbm.at[lo:hi, :], sem_o.at[n])

    xa_copy = x_rows(0, 0, RA)
    xb_copy = x_rows(1, RA, TQ)
    x_copies = [x_rows(1 + t, t * TQ, (t + 1) * TQ) for t in range(1, NQT)]
    wka_copy = w_cols(0, D, D + 384)
    wkb_copy = w_cols(1, D + 384, 2 * D)
    wq_copy = w_cols(2, 0, D)
    wv_copy = w_cols(3, 2 * D, 3 * D)
    late_copies = [
        pltpu.make_async_copy(src, dst, sem_w.at[4 + n])
        for n, (src, dst) in enumerate(
            [(wg_hbm, wg_ref), (wu_hbm, wu_ref), (wd_hbm, wd_ref), (wo_hbm, wo_ref)])
    ]

    z_ref[0] = 0
    for cp in [xa_copy, wka_copy, xb_copy, wkb_copy] + x_copies + [wq_copy, wv_copy]:
        cp.start()

    def layer_norm(lo, hi):
        x = x_ref[lo:hi, :].astype(f32)
        mean = jnp.mean(x, axis=-1, keepdims=True)
        xc = x - mean
        var = jnp.mean(xc * xc, axis=-1, keepdims=True)
        xn_ref[lo:hi, :] = (xc * lax.rsqrt(var + EPS)).astype(bf16)

    def wk_prep(j0, j1):
        for j in range(j0, j1):
            wk_ref[:, j * 128:(j + 1) * 128] = wqkv_ref[:, D + 120 * j:D + 120 * j + 128]

    def k_proj(lo, hi, j0, j1):
        kk = jnp.dot(xn_ref[lo:hi, :], wk_ref[:, j0 * 128:j1 * 128],
                     preferred_element_type=f32).astype(bf16)
        for j in range(j0, j1):
            k_ref[j, lo:hi, :] = kk[:, (j - j0) * 128:(j - j0 + 1) * 128]

    def k_split(lo, hi, j0, j1, parts):
        q = (hi - lo) // parts
        for p in range(parts):
            k_proj(lo + p * q, lo + (p + 1) * q, j0, j1)

    row24 = lax.broadcasted_iota(jnp.int32, (VW, TQ), 0)

    def qv_proj(t):
        lo, hi = t * TQ, (t + 1) * TQ
        qv = lax.dot_general(wqvt_ref[0:2 * D + KX, :], xn_ref[lo:hi, :], _NT,
                             preferred_element_type=f32)
        qt_ref[t, 0:D, :] = qv[0:D] * QSCALE
        for h in range(H):
            w = 8 * ((DH * h) // 8)
            ones_row = 0 if h % 2 else VW - 1
            vt_ref[h, :, lo:hi] = jnp.where(row24 == ones_row, 1.0, qv[D + w:D + w + VW])
        kx = jnp.concatenate([jnp.zeros((128 - KX, TQ), f32), qv[2 * D:2 * D + KX]], axis=0)
        k_ref[NKT - 1, lo:hi, :] = kx.T.astype(bf16)

    s1_ref[...] = jnp.zeros((S, TQ), f32)
    m1_ref[...] = jnp.zeros((1, TQ), f32)

    xa_copy.wait()
    layer_norm(0, RA)
    wka_copy.wait()
    wk_prep(0, 3)
    k_proj(0, RA, 0, 3)
    xb_copy.wait()
    wkb_copy.wait()
    layer_norm(RA, TQ)
    wk_prep(3, 5)
    k_proj(0, RA, 3, 5)
    for t in range(1, NQT):
        x_copies[t - 1].wait()
        if t == 1:
            k_proj(RA, TQ, 0, 4)
            k_split(RA, TQ, 4, 5, 4)
        else:
            k_split((t - 1) * TQ, t * TQ, 3, 5, 2)
        layer_norm(t * TQ, (t + 1) * TQ)
        k_split(t * TQ, (t + 1) * TQ, 0, 3, 4)
    wq_copy.wait()
    wv_copy.wait()
    for cp in late_copies:
        cp.start()
    k_split((NQT - 1) * TQ, NQT * TQ, 3, 5, 2)
    wqvt_ref[0:D, :] = wqkv_ref[:, 0:D].T
    wqvt_ref[D:2 * D, :] = wqkv_ref[:, 2 * D:3 * D].T
    wqvt_ref[2 * D:2 * D + KX, :] = wqkv_ref[:, 2 * D - 128:2 * D].T[128 - KX:128]
    for t in range(NQT):
        qv_proj(t)
    for cp in late_copies:
        cp.wait()

    row128 = lax.broadcasted_iota(jnp.int32, (128, TQ), 0)
    row8 = lax.broadcasted_iota(jnp.int32, (8, TQ), 0)

    def q_weights(h, t):
        j = h // HPT
        start = jnp.minimum(120 * j, D - 128)
        o = DH * h - start
        win = qt_ref[t, pl.ds(pl.multiple_of(start, 8), 128), :]
        mask = (row128 >= o) & (row128 < o + DH)
        return jnp.where(mask, win, 0.0).astype(bf16), j

    def qk_chunk(wq, j, c, s_ref, mx):
        s = jnp.dot(k_ref[j, c * CK:(c + 1) * CK, :], wq, preferred_element_type=f32)
        s_ref[c * CK:(c + 1) * CK, :] = s
        return jnp.maximum(mx, jnp.max(s.reshape(CK // 8, 8, TQ), axis=0))

    def pv_chunk(h, c, s_ref, m, acc):
        p = jnp.exp2(s_ref[c * CK:(c + 1) * CK, :] - m).astype(bf16)
        return acc + jnp.dot(vt_ref[h, :, c * CK:(c + 1) * CK], p, preferred_element_type=f32)

    def finish(h, t, odd, acc):
        w = DH * h - (4 if odd else 0)
        if not isinstance(h, int):
            w = pl.multiple_of(w, 8)
        den = acc[0:1] if odd else acc[VW - 1:VW]
        o = acc * (1.0 / den)
        if odd:
            pltpu.store(ot_ref.at[t, pl.ds(w, 8), :], o[0:8], mask=row8 >= 4)
            ot_ref[t, pl.ds(w + 8, 16), :] = o[8:VW]
        else:
            ot_ref[t, pl.ds(w, 16), :] = o[0:16]
            pltpu.store(ot_ref.at[t, pl.ds(w + 16, 8), :], o[16:VW], mask=row8 < 4)

    neg = jnp.full((8, TQ), -jnp.inf, f32)
    bufs = ((s0_ref, m0_ref), (s1_ref, m1_ref))

    def stream(curs, nxts, hooks=None):
        n_items = max(len(curs), len(nxts))
        for g in range(n_items * NCK + LAG):
            if hooks and g in hooks:
                hooks[g]()
            n, c = divmod(g, NCK)
            if n < len(nxts):
                s_nxt, m_nxt = bufs[n % 2]
                if c == 0:
                    wq, j = q_weights(nxts[n][0], nxts[n][1])
                    mx = neg
                mx = qk_chunk(wq, j, c, s_nxt, mx)
                if c == NCK - 1:
                    m_nxt[...] = jnp.max(mx, axis=0, keepdims=True)
            n, c = divmod(g - LAG, NCK)
            if 0 <= n < len(curs):
                s_cur, m_cur = bufs[(n + 1) % 2]
                if c == 0:
                    m = m_cur[...]
                    acc = jnp.zeros((VW, TQ), f32)
                acc = pv_chunk(curs[n][0], c, s_cur, m, acc)
                if c == NCK - 1:
                    finish(*curs[n], acc)

    def attn_body(hb, carry):
        r0 = pl.multiple_of(hb * FR, FR)
        xn = xn_ref[pl.ds(r0, FR), :]
        ffn = {}

        def gate_up(i):
            g = jnp.dot(xn, wg_ref[:, i * FQ:(i + 1) * FQ], preferred_element_type=f32)
            u = jnp.dot(xn, wu_ref[:, i * FQ:(i + 1) * FQ], preferred_element_type=f32)
            ffn["hm"] = (g * jax.nn.sigmoid(g) * u).astype(bf16)

        def down(i):
            r = jnp.dot(ffn["hm"], wd_ref[i * FQ:(i + 1) * FQ, :], preferred_element_type=f32)
            ffn["out"] = ffn["out"] + r if i else r

        def piece(i):
            down(i - 1)
            gate_up(i)

        hooks = {2 * NCK * i + 1: (lambda i=i: piece(i)) for i in range(1, F // FQ)}
        items = [(hb * HPB + a, t, a % 2 == 1) for a in range(HPB) for t in range(NQT)]
        prev = (jnp.maximum(hb * HPB - 1, 1), NQT - 1, True)

        gate_up(0)
        stream([prev] + items[:-1], items, hooks)
        down(F // FQ - 1)
        part_ref[pl.ds(r0, FR), :] = x_ref[pl.ds(r0, FR), :].astype(f32) + ffn["out"]
        return carry

    lax.fori_loop(0, H // HPB, attn_body, 0)

    z = z_ref[0]
    m1_ref[...] = jnp.where(z == 0, m1_ref[...], s0_ref[pl.ds(pl.multiple_of(8 * z, 8), 1), :])
    stream([(H - 1, NQT - 1, True)], [])

    copies = []
    for t in range(NQT):
        parts = OSPLIT if t == NQT - 1 else 1
        rows = TQ // parts
        for p in range(parts):
            lo = t * TQ + p * rows
            o_t = ot_ref[t, :, p * rows:(p + 1) * rows].astype(bf16)
            attn = lax.dot_general(o_t, wo_ref[...], _TN, preferred_element_type=f32)
            out_ref[lo:lo + rows, :] = (part_ref[lo:lo + rows, :] + attn).astype(bf16)
            cp = o_rows(len(copies), lo, lo + rows)
            cp.start()
            copies.append(cp)
    for cp in copies:
        cp.wait()


@jax.jit
def pallas_parallel_sum__softmax_full_mha__swiglu_ffn__prompt_kernel(
    A_x: jax.Array,
    A_wqkv: jax.Array,
    A_wo: jax.Array,
    B_x: jax.Array,
    B_w_gate: jax.Array,
    B_w_up: jax.Array,
    B_w_down: jax.Array,
):
    del B_x
    bf16 = jnp.bfloat16
    f32 = jnp.float32
    any_spec = pl.BlockSpec(memory_space=pl.ANY)
    out = pl.pallas_call(
        _kernel,
        out_shape=jax.ShapeDtypeStruct((S, D), bf16),
        in_specs=[any_spec] * 6,
        out_specs=any_spec,
        scratch_shapes=[
            pltpu.VMEM((S, D), bf16),
            pltpu.VMEM((D, 3 * D), bf16),
            pltpu.VMEM((D, D), bf16),
            pltpu.VMEM((D, F), bf16),
            pltpu.VMEM((D, F), bf16),
            pltpu.VMEM((F, D), bf16),
            pltpu.VMEM((S, D), bf16),
            pltpu.VMEM((S, D), bf16),
            pltpu.VMEM((D, (NKT - 1) * 128), bf16),
            pltpu.VMEM((2 * D + 64, D), bf16),
            pltpu.VMEM((NKT, S, 128), bf16),
            pltpu.VMEM((NQT, D, TQ), f32),
            pltpu.VMEM((H, VW, S), f32),
            pltpu.VMEM((NQT, D, TQ), f32),
            pltpu.VMEM((S, D), f32),
            pltpu.VMEM((S, TQ), f32),
            pltpu.VMEM((S, TQ), f32),
            pltpu.VMEM((1, TQ), f32),
            pltpu.VMEM((1, TQ), f32),
            pltpu.SMEM((1,), jnp.int32),
            pltpu.SemaphoreType.DMA((NQT + 1,)),
            pltpu.SemaphoreType.DMA((8,)),
            pltpu.SemaphoreType.DMA((NQT - 1 + OSPLIT,)),
        ],
        compiler_params=pltpu.CompilerParams(vmem_limit_bytes=110 * 1024 * 1024),
    )(A_x.reshape(S, D), A_wqkv, A_wo, B_w_gate, B_w_up, B_w_down)
    return out.reshape(1, S, D)
```
